```python
import jax
import jax.numpy as jnp

def _softmax(x, axis=-1):
    return jax.nn.softmax(x, axis=axis)
def _gelu(x):
    return jax.nn.gelu(x, approximate=True)
def _silu(x):
    return jax.nn.silu(x)
def _sigmoid(x):
    return jax.nn.sigmoid(x)
def _layernorm(x, axis=-1, eps=1e-5):
    m = jnp.mean(x, axis=axis, keepdims=True)
    v = jnp.var(x, axis=axis, keepdims=True)
    return (x - m) / jnp.sqrt(v + eps)
def _scatter_add(tgt, idx, src, axis=0):
    return tgt.at[idx].add(src)
def _segment_sum(src, seg, n):
    return jax.ops.segment_sum(src, seg, n)
class _Rng:
    def __init__(self, key):
        self._k = key
    def _next(self):
        self._k, sub = jax.random.split(self._k)
        return sub
    def normal(self, shape):
        return jax.random.normal(self._next(), shape, dtype=jnp.bfloat16)
    def randint(self, lo, hi, shape):
        return jax.random.randint(self._next(), shape, lo, hi, dtype=jnp.int32)
    def uniform(self, shape, lo=0.0, hi=1.0):
        return jax.random.uniform(self._next(), shape, jnp.bfloat16, lo, hi)
    def permutation(self, n):
        return jax.random.permutation(self._next(), n)


kernel_name = 'interleave_layers__sliding_local_dilated__glu_gated_geglu__prompt'

def setup_inputs():
    _rng = _Rng(jax.random.key(int.from_bytes(__import__("os").urandom(4), "little")))
    _w = (lambda a: (lambda t: t.astype(jnp.bfloat16) if jnp.issubdtype(t.dtype, jnp.floating) else t)(jnp.asarray(a)))
    def _A_setup():
        B, S, D = 1, 2048, 576
        return {
            "x": _w((lambda *s: _rng.normal(s) * 0.05)(B, S, D)),
            "wqkv": _w((lambda *s: _rng.normal(s) * 0.05)(D, 3 * D)),
            "wo": _w((lambda *s: _rng.normal(s) * 0.05)(D, D)),
        }
    _A_in = _A_setup()

    def _B_setup():
        B, S, Dm, Df = 1, 2048, 576, 4608
        return {
            "x": _w((lambda *s: _rng.normal(s) * 0.05)(B, S, Dm)),
            "w_gate": _w((lambda *s: _rng.normal(s) * 0.05)(Dm, Df) * (Dm ** -0.5)),
            "w_up": _w((lambda *s: _rng.normal(s) * 0.05)(Dm, Df) * (Dm ** -0.5)),
            "w_down": _w((lambda *s: _rng.normal(s) * 0.05)(Df, Dm) * (Df ** -0.5)),
        }
    _B_in = _B_setup()

    return {
        "A_x": _A_in["x"],
        "A_wqkv": _A_in["wqkv"],
        "A_wo": _A_in["wo"],
        "B_x": _B_in["x"],
        "B_w_gate": _B_in["w_gate"],
        "B_w_up": _B_in["w_up"],
        "B_w_down": _B_in["w_down"],
    }

def reference(A_x, A_wqkv, A_wo, B_x, B_w_gate, B_w_up, B_w_down):
    def _A_ref(x, wqkv, wo):
        B, S, D = x.shape
        H = 32; Dh = D // H
        W, dil = 8, 2
        qkv = (lambda x, *d: x.transpose(*d))((x @ wqkv).reshape(B, S, 3, H, Dh), 2, 0, 3, 1, 4)
        q, k, v = qkv[0], qkv[1], qkv[2]
        scale = Dh ** -0.5
        pos = jnp.arange(S)
        off = jnp.arange(W) * dil
        idx = pos[:, None] - off[None, :]
        mask = idx >= 0
        idx_c = jnp.where(mask, idx, 0).reshape(-1)
        kg = k[:, :, idx_c, :].reshape(B, H, S, W, Dh)
        vg = v[:, :, idx_c, :].reshape(B, H, S, W, Dh)
        logits = jnp.einsum("bhsd,bhswd->bhsw", q, kg) * scale
        logits = jnp.where(mask[None, None, :, :], logits, -1e9)
        attn = _softmax(logits, axis=-1)
        o = jnp.einsum("bhsw,bhswd->bhsd", attn, vg)
        return (lambda x, *d: x.transpose(*d))(o, 0, 2, 1, 3).reshape(B, S, D) @ wo

    def _B_ref(x, w_gate, w_up, w_down):
        g = jnp.einsum("bsd,df->bsf", x, w_gate)
        u = jnp.einsum("bsd,df->bsf", x, w_up)
        h = _gelu(g) * u
        return jnp.einsum("bsf,fd->bsd", h, w_down)

    x = A_x
    x = x + _A_ref(_layernorm(x, axis=-1), A_wqkv, A_wo)
    x = x + _B_ref(_layernorm(x, axis=-1), B_w_gate, B_w_up, B_w_down)
    x = x + _A_ref(_layernorm(x, axis=-1), A_wqkv, A_wo)
    x = x + _B_ref(_layernorm(x, axis=-1), B_w_gate, B_w_up, B_w_down)
    return x
```

```python
import functools
import jax
import jax.numpy as jnp
import numpy as np
import jax.experimental.pallas as pl
import jax.experimental.pallas.tpu as pltpu

S, D, DP = 2048, 576, 640
H, DH, W, DIL = 32, 18, 8, 2
DF = 4608
PAD = 16
NEG = -1e30
LOG2E = 1.4426950408889634
F32, BF16 = jnp.float32, jnp.bfloat16
NT = (((1,), (1,)), ((), ()))


def _ln_t(x):
    m = jnp.mean(x, axis=0, keepdims=True)
    xc = x - m
    v = jnp.mean(xc * xc, axis=0, keepdims=True)
    return xc * jax.lax.rsqrt(v + 1e-5)


def _gelu(x):
    c = 0.7978845608028654
    return 0.5 * x * (1.0 + jnp.tanh(c * (x + 0.044715 * (x * x * x))))


def make_kernel(T=256, RS=32, FB=1536, tmode=0, NL=2, pin=1, pin0=0.0, pin1=0.66, wof=1, dord=0):
    NC = S // T
    NF = DF // FB
    NSB = T // RS

    def kernel(xT_hbm, wqkv_hbm, wo_hbm, wg_hbm, wu_hbm, wdT_hbm, outT_hbm,
               xin, xa, xb, outs, wqkv_raw, wo_raw, w32, wqkvP, woTP, wg, wu, wdT,
               q_s, k_s, v_s, xnA, xnB_s, o_s, zs, sems, osem):
        def cp_cols(src, dst, c0, n, sem):
            return pltpu.make_async_copy(src.at[:, pl.ds(c0, n)], dst.at[:, pl.ds(c0, n)], sem)

        cp_x0 = cp_cols(xT_hbm, xin, 0, 2 * T, sems.at[0])
        cp_wqkv = pltpu.make_async_copy(wqkv_hbm, wqkv_raw, sems.at[1])
        cp_wo = pltpu.make_async_copy(wo_hbm, wo_raw, sems.at[2])
        cp_x1 = cp_cols(xT_hbm, xin, 2 * T, S - 2 * T, sems.at[3])
        cp_g = [cp_cols(wg_hbm, wg, f * FB, FB, sems.at[4 + 3 * f]) for f in range(NF)]
        cp_u = [cp_cols(wu_hbm, wu, f * FB, FB, sems.at[5 + 3 * f]) for f in range(NF)]
        cp_d = [cp_cols(wdT_hbm, wdT, f * FB, FB, sems.at[6 + 3 * f]) for f in range(NF)]
        order = [cp_x0, cp_wqkv, cp_wo, cp_g[0], cp_u[0], cp_x1]
        for f in range(NF):
            if f + 1 < NF:
                order += [cp_d[f], cp_g[f + 1], cp_u[f + 1]] if dord == 0 else [cp_g[f + 1], cp_u[f + 1], cp_d[f]]
            else:
                order += [cp_d[f]]
        for c in order:
            c.start()

        def out_copy(c):
            c0 = pl.multiple_of(c * T, T)
            return pltpu.make_async_copy(outs.at[:, pl.ds(c0, T)], outT_hbm.at[:, pl.ds(c0, T)], osem)

        zs[0] = 0
        k_s[pl.ds(0, PAD), :] = jnp.zeros((PAD, DP), F32)
        v_s[pl.ds(0, PAD), :] = jnp.zeros((PAD, DP), F32)

        cp_x0.wait()
        xb[:, 0:2 * T] = xin[:, 0:2 * T].astype(F32)

        cp_wqkv.wait()
        for j in range(14):
            ncol = min(128, 3 * D - j * 128)
            blk = wqkv_raw[:, j * 128:j * 128 + ncol].astype(F32)
            if ncol < 128:
                blk = jnp.concatenate([blk, jnp.zeros((D, 128 - ncol), F32)], axis=1)
            blk = jnp.concatenate([blk, jnp.zeros((DP - D, 128), F32)], axis=0)
            for t in range(5):
                w32[t, pl.ds(j * 128, 128), :] = blk[t * 128:(t + 1) * 128, :].T
        for p in range(3):
            for d in range(DH):
                dst = (p * 16 + d) if d < 16 else (48 + p * 2 + d - 16)
                for t in range(5):
                    rows = w32[t, pl.ds(p * D + d, H, stride=DH), :]
                    wqkvP[pl.ds(dst * H, H), t * 128:(t + 1) * 128] = rows.astype(BF16)
        cp_wo.wait()
        for t in range(5):
            ncol = min(128, D - t * 128)
            blk = wo_raw[:, t * 128:t * 128 + ncol].astype(F32)
            if ncol < 128:
                blk = jnp.concatenate([blk, jnp.zeros((D, 128 - ncol), F32)], axis=1)
            w32[t, pl.ds(0, D), :] = blk
            for d in range(DH):
                w32[t, pl.ds(D + d * H, H), :] = w32[t, pl.ds(d, H, stride=DH), :]
            w32[t, pl.ds(2 * D, 64), :] = jnp.zeros((64, 128), F32)
            for j in range(5):
                pb = w32[t, pl.ds(D + j * 128, 128), :]
                nrow = min(128, D - t * 128)
                woTP[pl.ds(t * 128, nrow), j * 128:(j + 1) * 128] = pb.T[0:nrow, :].astype(BF16)

        def ln_rows(xc):
            if tmode == 0:
                return _ln_t(xc).T.astype(BF16)
            return _ln_t(xc).astype(BF16).T

        lane = jax.lax.broadcasted_iota(jnp.int32, (T, 128), 1)
        lo_mask = lane < 64

        def qkv_part(c0):
            qkv = jax.lax.dot_general(xnA[...], wqkvP[:, 0:D], NT, preferred_element_type=F32)
            t12 = qkv[:, 1536:1664]
            q_s[pl.ds(0, T), 0:512] = qkv[:, 0:512]
            q_s[pl.ds(0, T), 512:640] = jnp.where(lo_mask, t12, 0.0)
            k_s[pl.ds(c0 + PAD, T), 0:512] = qkv[:, 512:1024]
            k_s[pl.ds(c0 + PAD, T), 512:640] = pltpu.roll(t12, 64, axis=1)
            v_s[pl.ds(c0 + PAD, T), 0:512] = qkv[:, 1024:1536]
            v_s[pl.ds(c0 + PAD, T), 512:576] = qkv[:, 1664:1728]
            v_s[pl.ds(c0 + PAD, T), 576:640] = jnp.zeros((T, 64), F32)

        def att_block(c0, sb):
            base = c0 + sb * RS
            q = q_s[pl.ds(sb * RS, RS), :]
            row = jax.lax.broadcasted_iota(jnp.int32, (RS, 128), 0) + base
            kk = k_s[pl.ds(base, RS + PAD), :]
            logits = []
            for w in range(W):
                o0 = PAD - DIL * w
                p = q * kk[o0:o0 + RS, :]
                s = p[:, 0:128] + p[:, 128:256] + p[:, 256:384] + p[:, 384:512] + p[:, 512:640]
                s = s + pltpu.roll(s, 64, axis=1)
                s = s + pltpu.roll(s, 32, axis=1)
                if w > 0:
                    s = jnp.where(row >= DIL * w, s, NEG)
                logits.append(s)
            m = logits[0]
            for w in range(1, W):
                m = jnp.maximum(m, logits[w])
            cs = LOG2E * DH ** -0.5
            es = [jnp.exp2((l - m) * cs) for l in logits]
            den = es[0]
            for w in range(1, W):
                den = den + es[w]
            inv = 1.0 / den
            vv = v_s[pl.ds(base, RS + PAD), :]
            o = None
            for w in range(W):
                o0 = PAD - DIL * w
                e5 = jnp.concatenate([es[w]] * 5, axis=1)
                t = e5 * vv[o0:o0 + RS, :]
                o = t if o is None else o + t
            o = o * jnp.concatenate([inv] * 5, axis=1)
            o_s[pl.ds(sb * RS, RS), :] = o.astype(BF16)

        def pin_q(val):
            off = pl.multiple_of(T + zs[0], 8)
            q_s[pl.ds(off, 8), 0:128] = val

        def pin_b(val):
            off = pl.multiple_of(T + zs[0], 16)
            xnB_s[pl.ds(off, 16), 0:128] = val

        def body(s, doA, doB, doNext, first=False):
            if doA:
                a0 = pl.multiple_of((s % NC) * T, T)
                qkv_part(a0)
            if doNext:
                n0 = pl.multiple_of(((s + 1) % NC) * T, T)
                xnA[...] = ln_rows(xb[:, pl.ds(n0, T)])
                if pin and doA:
                    zoff = pl.multiple_of(zs[0], 16)
                    pin_q(xnA[pl.ds(zoff, 16), 0:128].astype(F32)[0:8, :])
            if doB:
                b0 = pl.multiple_of(((s - 1) % NC) * T, T)
                acc = xa[:, pl.ds(b0, T)]
                xnB_s[pl.ds(0, T), :] = ln_rows(acc)

            def att_tail():
                yT = jax.lax.dot_general(woTP[:, 0:D], o_s[:, 0:D], NT, preferred_element_type=F32)
                xa[:, pl.ds(a0, T)] = xb[:, pl.ds(a0, T)] + yT

            done = 0
            for f in range(NF):
                if doB:
                    xnB = xnB_s[pl.ds(0, T), :]
                    if first:
                        cp_g[f].wait()
                        cp_u[f].wait()
                    g = jnp.dot(xnB, wg[:, f * FB:(f + 1) * FB], preferred_element_type=F32)
                    u = jnp.dot(xnB, wu[:, f * FB:(f + 1) * FB], preferred_element_type=F32)
                    h = (_gelu(g) * u).astype(BF16)
                if doA:
                    for sb in range(NSB):
                        pos = pin0 + (pin1 - pin0) * sb / NSB
                        if int(pos * NF) != f:
                            continue
                        if doB and pin:
                            col = int((pos * NF - f) * FB) // 128 * 128
                            pin_q(g[0:8, col:col + 128])
                        att_block(a0, sb)
                        done += 1
                    if done == NSB and wof:
                        done += 1
                        att_tail()
                        if doB and pin and f + 1 < NF:
                            zc = pl.multiple_of(a0 + zs[0], 128)
                            pin_b(xa[0:16, pl.ds(zc, 128)].astype(BF16))
                if doB:
                    if first:
                        cp_d[f].wait()
                    acc = acc + jax.lax.dot_general(wdT[:, f * FB:(f + 1) * FB], h, NT, preferred_element_type=F32)
            if doA and not wof:
                att_tail()
            if doB:
                xb[:, pl.ds(b0, T)] = acc
                outs[:, pl.ds(b0, T)] = acc.astype(BF16)
                @pl.when(s - 1 >= (NL - 1) * NC)
                def _():
                    out_copy(s - 1 - (NL - 1) * NC).start()

        xnA[...] = ln_rows(xb[:, pl.ds(0, T)])
        body(0, True, False, True)
        cp_x1.wait()

        def cvt(i, _):
            c0 = pl.multiple_of(i * T, T)
            xb[:, pl.ds(c0, T)] = xin[:, pl.ds(c0, T)].astype(F32)
            return None
        jax.lax.fori_loop(2, NC, cvt, None)
        body(1, True, True, True, first=True)

        def loop_body(s, _):
            body(s, True, True, True)
            return None
        jax.lax.fori_loop(2, NL * NC, loop_body, None)
        body(NL * NC, False, True, False)
        for c in range(NC):
            out_copy(c).wait()

    return kernel


def build(**cfg):
    cfg = dict(cfg)
    flags = cfg.pop("flags", None)
    kern = make_kernel(**cfg)
    T = cfg.get("T", 256)

    @jax.jit
    def fn(A_x, A_wqkv, A_wo, B_x, B_w_gate, B_w_up, B_w_down):
        xT = A_x.reshape(S, D).T
        wdT = B_w_down.T
        hbm = pl.BlockSpec(memory_space=pltpu.HBM)
        outT = pl.pallas_call(
            kern,
            out_shape=jax.ShapeDtypeStruct((D, S), BF16),
            in_specs=[hbm] * 6,
            out_specs=hbm,
            scratch_shapes=[
                pltpu.VMEM((D, S), BF16),
                pltpu.VMEM((D, S), F32),
                pltpu.VMEM((D, S), F32),
                pltpu.VMEM((D, S), BF16),
                pltpu.VMEM((D, 3 * D), BF16),
                pltpu.VMEM((D, D), BF16),
                pltpu.VMEM((5, 1792, 128), F32),
                pltpu.VMEM((3 * D, DP), BF16),
                pltpu.VMEM((D, DP), BF16),
                pltpu.VMEM((D, DF), BF16),
                pltpu.VMEM((D, DF), BF16),
                pltpu.VMEM((D, DF), BF16),
                pltpu.VMEM((T + 8, DP), F32),
                pltpu.VMEM((S + PAD, DP), F32),
                pltpu.VMEM((S + PAD, DP), F32),
                pltpu.VMEM((T, D), BF16),
                pltpu.VMEM((T + 16, D), BF16),
                pltpu.VMEM((T, DP), BF16),
                pltpu.SMEM((1,), jnp.int32),
                pltpu.SemaphoreType.DMA((4 + 3 * (DF // cfg.get('FB', 1536)),)),
                pltpu.SemaphoreType.DMA(()),
            ],
            compiler_params=pltpu.CompilerParams(vmem_limit_bytes=110 * 1024 * 1024, flags=flags),
        )(xT, A_wqkv, A_wo, B_w_gate, B_w_up, wdT)
        return outT.T.reshape(1, S, D)
    return fn


_kernel_fn = build()


@jax.jit
def pallas_interleave_layers__sliding_local_dilated__glu_gated_geglu__prompt_kernel(
    A_x: jax.Array,
    A_wqkv: jax.Array,
    A_wo: jax.Array,
    B_x: jax.Array,
    B_w_gate: jax.Array,
    B_w_up: jax.Array,
    B_w_down: jax.Array,
):
    return _kernel_fn(A_x, A_wqkv, A_wo, B_x, B_w_gate, B_w_up, B_w_down)
```

```python
import contextlib
import jax
import jax.numpy as jnp
import jax.experimental.pallas as pl
import jax.experimental.pallas.tpu as pltpu

S, D, DP = 2048, 576, 640
H, DH, W, DIL = 32, 18, 8, 2
DF = 4608
PAD = 16
NEG = -1e30
LOG2E = 1.4426950408889634
F32, BF16 = jnp.float32, jnp.bfloat16
NT = (((1,), (1,)), ((), ()))


def _ln_t(x):
    m = jnp.mean(x, axis=0, keepdims=True)
    xc = x - m
    v = jnp.mean(xc * xc, axis=0, keepdims=True)
    return xc * jax.lax.rsqrt(v + 1e-5)


def _ln_rows(xc):
    return _ln_t(xc).T.astype(BF16)


def _gelu(x):
    c = 0.7978845608028654
    return 0.5 * x * (1.0 + jnp.tanh(c * (x + 0.044715 * (x * x * x))))


ORDER = 'xin xa xb outs wqkv_raw wo_raw w32 wqkvP woTP wg wu wdT q k v xnA xnB xnC o zs sems osem'.split()


def make_kernel(names, T=256, RS=16, FB=1536, NL=2, pin0=0.0, pin1=0.66, PR=16,
                scopes=0, NCV=4, dma6=0, p6=0, v6=0, pinb=0, nopeel=0, lnA=0, lnB=-1, split0=1, cvt_in1=1, ord1=1):
    NC = S // T
    NF = DF // FB
    NSB = T // RS
    assert NF == 3

    def kernel(xT_hbm, wqkv_hbm, wo_hbm, wg_hbm, wu_hbm, wdT_hbm, outT_hbm, *scratch):
        sc_ = dict(zip(names, scratch))
        (xin, xa, xb, outs, wqkv_raw, wo_raw, w32, wqkvP, woTP, wg, wu, wdT,
         q_s, k_s, v_s, xnA, xnB_s, xnC, o_s, zs, sems, osem) = [sc_.get(n) for n in ORDER]
        def cp_cols(src, dst, c0, n, sem):
            return pltpu.make_async_copy(src.at[:, pl.ds(c0, n)], dst.at[pl.ds(0, D), pl.ds(c0, n)], sem)

        QP = [(0, 640), (640, 512), (1152, 576)]
        cp_x0 = cp_cols(xT_hbm, xin, 0, T, sems.at[0])
        cp_x1 = cp_cols(xT_hbm, xin, T, T, sems.at[1])
        cp_x2 = cp_cols(xT_hbm, xin, 2 * T, S - 2 * T, sems.at[2])
        cp_q = [cp_cols(wqkv_hbm, wqkv_raw, c0, n, sems.at[3 + i]) for i, (c0, n) in enumerate(QP)]
        cp_wo = pltpu.make_async_copy(wo_hbm, wo_raw, sems.at[6])
        cp_g = [cp_cols(wg_hbm, wg, f * FB, FB, sems.at[7 + 3 * f]) for f in range(NF)]
        cp_u = [cp_cols(wu_hbm, wu, f * FB, FB, sems.at[8 + 3 * f]) for f in range(NF)]
        cp_d = [cp_cols(wdT_hbm, wdT, f * FB, FB, sems.at[9 + 3 * f]) for f in range(NF)]
        order = [cp_x0, cp_q[0], cp_q[1], cp_q[2], cp_wo, cp_x1, cp_x2, cp_g[0], cp_u[0],
                 cp_g[1], cp_u[1], cp_d[0], cp_g[2], cp_u[2], cp_d[1], cp_d[2]]
        if dma6:
            class _N:
                def wait(self):
                    pass
            cp_q = [pltpu.make_async_copy(wqkv_hbm, wqkv_raw, sems.at[3]), _N(), _N()]
            order = [order[0]] + order[4:]
            order.insert(1, cp_q[0])
        for c in order:
            c.start()

        def out_copy(c):
            c0 = pl.multiple_of(c * T, T)
            return pltpu.make_async_copy(outs.at[:, pl.ds(c0, T)], outT_hbm.at[:, pl.ds(c0, T)], osem)

        def cvt(c):
            xb[:, c * T:(c + 1) * T] = xin[:, c * T:(c + 1) * T].astype(F32)

        zs[0] = 0
        for j in range(5):
            k_s[j, pl.ds(T, PAD), :] = jnp.zeros((PAD, 128), F32)
            v_s[j, pl.ds(T, PAD), :] = jnp.zeros((PAD, 128), F32)

        def transpose_blocks(j0, j1):
            for j in range(j0, j1):
                ncol = min(128, 3 * D - j * 128)
                blk = wqkv_raw[:, j * 128:j * 128 + ncol].astype(F32)
                if ncol < 128:
                    blk = jnp.concatenate([blk, jnp.zeros((D, 128 - ncol), F32)], axis=1)
                blk = jnp.concatenate([blk, jnp.zeros((DP - D, 128), F32)], axis=0)
                for t in range(5):
                    w32[t, pl.ds(j * 128, 128), :] = blk[t * 128:(t + 1) * 128, :].T

        def permute_part(p):
            for d in range(DH):
                dst = (p * 16 + d) if d < 16 else (48 + p * 2 + d - 16)
                for t in range(5):
                    rows = w32[t, pl.ds(p * D + d, H, stride=DH), :]
                    wqkvP[pl.ds(dst * H, H), t * 128:(t + 1) * 128] = rows.astype(BF16)

        def prep_wo():
            for t in range(5):
                ncol = min(128, D - t * 128)
                blk = wo_raw[:, t * 128:t * 128 + ncol].astype(F32)
                if ncol < 128:
                    blk = jnp.concatenate([blk, jnp.zeros((D, 128 - ncol), F32)], axis=1)
                w32[t, pl.ds(0, D), :] = blk
                for d in range(DH):
                    w32[t, pl.ds(D + d * H, H), :] = w32[t, pl.ds(d, H, stride=DH), :]
                w32[t, pl.ds(2 * D, 64), :] = jnp.zeros((64, 128), F32)
                for j in range(5):
                    pb = w32[t, pl.ds(D + j * 128, 128), :]
                    woTP[pl.ds(t * 128, ncol), j * 128:(j + 1) * 128] = pb.T[0:ncol, :].astype(BF16)

        lane = jax.lax.broadcasted_iota(jnp.int32, (T, 128), 1)
        lo_mask = lane < 64
        cs = LOG2E * DH ** -0.5

        def halo(c0):
            keep = c0 > 0
            for j in range(5):
                k_s[j, pl.ds(0, PAD), :] = jnp.where(keep, k_s[j, pl.ds(T, PAD), :], 0.0)
                v_s[j, pl.ds(0, PAD), :] = jnp.where(keep, v_s[j, pl.ds(T, PAD), :], 0.0)

        def proj(r0, n):
            return jax.lax.dot_general(xnA[...], wqkvP[pl.ds(r0, n), 0:D], NT, preferred_element_type=F32)

        def store_main(ref, r, j0, val, scale=None):
            for j in range(4):
                v = val[:, j0 + j * 128:j0 + (j + 1) * 128]
                ref[j, pl.ds(r, T), :] = v if scale is None else v * scale

        def store_qk_tail(t12):
            q_s[4, pl.ds(0, T), :] = jnp.where(lo_mask, t12 * cs, 0.0)
            k_s[4, pl.ds(PAD, T), :] = pltpu.roll(t12, 64, axis=1)

        def store_v_tail(vt):
            v_s[4, pl.ds(PAD, T), :] = jnp.concatenate([vt, jnp.zeros((T, 64), F32)], axis=1)

        def qkv_part(c0=None):
            qkv = proj(0, 3 * D)
            if c0 is not None:
                halo(c0)
            if v6:
                for j in range(4):
                    q_s[j, pl.ds(0, T), :] = qkv[:, j * 128:(j + 1) * 128] * cs
                    k_s[j, pl.ds(PAD, T), :] = qkv[:, 512 + j * 128:512 + (j + 1) * 128]
                    v_s[j, pl.ds(PAD, T), :] = qkv[:, 1024 + j * 128:1024 + (j + 1) * 128]
                store_qk_tail(qkv[:, 1536:1664])
                store_v_tail(qkv[:, 1664:1728])
                return
            store_main(q_s, 0, 0, qkv, cs)
            store_main(k_s, PAD, 512, qkv)
            store_main(v_s, PAD, 1024, qkv)
            store_qk_tail(qkv[:, 1536:1664])
            store_v_tail(qkv[:, 1664:1728])

        def att_block(c0, sb):
            base = sb * RS
            q = [q_s[j, pl.ds(base, RS), :] for j in range(5)]
            logits = []
            for w in range(W):
                o0 = PAD - DIL * w
                s = None
                for j in range(5):
                    p = q[j] * k_s[j, pl.ds(base + o0, RS), :]
                    s = p if s is None else s + p
                s = s + pltpu.roll(s, 64, axis=1)
                s = s + pltpu.roll(s, 32, axis=1)
                if base < DIL * w:
                    row = jax.lax.broadcasted_iota(jnp.int32, (RS, 128), 0) + (base + c0)
                    s = jnp.where(row >= DIL * w, s, NEG)
                logits.append(s)
            m = logits[0]
            for w in range(1, W):
                m = jnp.maximum(m, logits[w])
            es = [jnp.exp2(l - m) for l in logits]
            den = es[0]
            for w in range(1, W):
                den = den + es[w]
            inv = 1.0 / den
            for j in range(5):
                o = None
                for w in range(W):
                    o0 = PAD - DIL * w
                    t = es[w] * v_s[j, pl.ds(base + o0, RS), :]
                    o = t if o is None else o + t
                o_s[pl.ds(base, RS), j * 128:(j + 1) * 128] = (o * inv).astype(BF16)

        def att_tail(a0):
            yT = jax.lax.dot_general(woTP[:, 0:D], o_s[:, 0:D], NT, preferred_element_type=F32)
            xa_new = xb[:, pl.ds(a0, T)] + yT
            xa[:, pl.ds(a0, T)] = xa_new
            return xa_new

        def pin_q(val):
            q_s[0, pl.ds(pl.multiple_of(T + zs[0], 8), 8), :] = val

        def pin_d(val):
            wdT[pl.ds(pl.multiple_of(D + zs[0], 16), 16), 0:128] = val

        def fence(ref):
            return ref[pl.ds(pl.multiple_of(zs[0], 16), 16), 0:128]

        def body(s, doA, doB, doNext, first=False):
            if doA:
                a0 = pl.multiple_of((s % NC) * T, T)
                if v6:
                    qkv_part(a0)
                else:
                    halo(a0)
                    qkv_part()
            if first:
                for c in range(NCV, NC):
                    cvt(c)
            if doNext:
                n0 = pl.multiple_of(((s + 1) % NC) * T, T)

            def ln_next():
                xnA[...] = _ln_rows(xb[:, pl.ds(n0, T)])

            if doNext and lnA < 0:
                ln_next()
                pin_q(fence(xnA).astype(F32)[0:8, :])
            if doB:
                b0 = pl.multiple_of(((s - 1) % NC) * T, T)
                acc = xa[:, pl.ds(b0, T)]
                if lnB < 0:
                    xnB_s[pl.ds(0, T), :] = _ln_rows(acc)
                else:
                    xnB_s[pl.ds(0, T), :] = xnC[...]

            hs = {}
            state = {"done": 0, "xa_new": None}

            def gate_up(f):
                xnB = xnB_s[pl.ds(0, T), :]
                if first:
                    for c in ([cp_g[0], cp_u[0]], [cp_g[1], cp_u[1]], [cp_g[2], cp_u[2]])[f]:
                        c.wait()
                g = jnp.dot(xnB, wg[:, f * FB:(f + 1) * FB], preferred_element_type=F32)
                u = jnp.dot(xnB, wu[:, f * FB:(f + 1) * FB], preferred_element_type=F32)
                hs[f] = (_gelu(g) * u).astype(BF16)
                return g

            def attention(f, g):
                for sb in range(NSB):
                    pos = pin0 + (pin1 - pin0) * sb / NSB
                    if int(pos * NF) != f:
                        continue
                    if g is not None and (sb * RS) % PR == 0:
                        col = int((pos * NF - f) * FB) // 128 * 128
                        pin_q(g[0:8, col:col + 128])
                    att_block(a0, sb)
                    state["done"] += 1
                if state["done"] == NSB:
                    state["done"] += 1
                    state["xa_new"] = att_tail(a0)
                    if pinb and f + 1 < NF:
                        zc = pl.multiple_of(a0 + zs[0], 128)
                        xnB_s[pl.ds(pl.multiple_of(T + zs[0], 16), 16), 0:128] = xa[0:16, pl.ds(zc, 128)].astype(BF16)

            def down(f, acc):
                if doNext and lnA == f:
                    ln_next()
                    pin_d(fence(xnA))
                if doA and lnB == f:
                    xnC[...] = _ln_rows(state["xa_new"])
                    pin_d(fence(xnC))
                if first:
                    cp_d[f].wait()
                return acc + jax.lax.dot_general(wdT[pl.ds(0, D), f * FB:(f + 1) * FB], hs[f], NT, preferred_element_type=F32)

            if not doB:
                for f in range(NF):
                    attention(f, None)
            if doB:
                if first and ord1:
                    g = gate_up(0)
                    attention(0, g)
                    g = gate_up(1); attention(1, g)
                    acc = down(0, acc)
                    g = gate_up(2); attention(2, g)
                    acc = down(1, acc)
                    acc = down(2, acc)
                else:
                    for f in range(NF):
                        g = gate_up(f)
                        if doA:
                            attention(f, g)
                        acc = down(f, acc)
                xb[:, pl.ds(b0, T)] = acc
                outs[:, pl.ds(b0, T)] = acc.astype(BF16)
                @pl.when(s - 1 >= (NL - 1) * NC)
                def _():
                    out_copy(s - 1 - (NL - 1) * NC).start()

        sc = (lambda n: jax.named_scope(n)) if scopes else (lambda n: contextlib.nullcontext())
        if p6:
            cp_x0.wait()
            cp_x1.wait()
            cvt(0)
            cvt(1)
            for c in cp_q:
                c.wait()
            transpose_blocks(0, 14)
            for p in range(3):
                permute_part(p)
            cp_wo.wait()
            prep_wo()
            xnA[...] = _ln_rows(xb[:, 0:T])
            body(0, True, False, False)
            xnA[...] = _ln_rows(xb[:, T:2 * T])
        else:
            with sc('s0_waitx'):
                cp_x0.wait()
            cvt(0)
            xnA[...] = _ln_rows(xb[:, 0:T])
            with sc('s1_waitq0'):
                cp_q[0].wait()
            transpose_blocks(0, 5)
            permute_part(0)
            if split0:
                store_main(q_s, 0, 0, proj(0, 512), cs)
            cp_q[1].wait()
            transpose_blocks(5, 9)
            permute_part(1)
            if split0:
                store_main(k_s, PAD, 0, proj(512, 512))
            with sc('s2_waitq2'):
                cp_q[2].wait()
            transpose_blocks(9, 14)
            permute_part(2)
            cp_wo.wait()
            cp_x1.wait()
            for j in range(5):
                k_s[j, pl.ds(0, PAD), :] = jnp.zeros((PAD, 128), F32)
                v_s[j, pl.ds(0, PAD), :] = jnp.zeros((PAD, 128), F32)
            if split0:
                rest = proj(1024, 704)
                store_qk_tail(rest[:, 512:640])
                store_main(v_s, PAD, 0, rest)
                store_v_tail(rest[:, 640:704])
            else:
                qkv_part()
            prep_wo()
            cvt(1)
            xnA[...] = _ln_rows(xb[:, T:2 * T])
            for sb in range(NSB):
                att_block(0, sb)
            xa_new = att_tail(0)
            if lnB >= 0:
                xnC[...] = _ln_rows(xa_new)

        cp_x2.wait()

        def cvt_d(i, _):
            c0 = pl.multiple_of(i * T, T)
            xb[:, pl.ds(c0, T)] = xin[:, pl.ds(c0, T)].astype(F32)
            return None
        jax.lax.fori_loop(2, NCV, cvt_d, None)
        if nopeel:
            for c in cp_g + cp_u + cp_d:
                c.wait()
        else:
            with sc('s5_step1'):
                body(1, True, True, True, first=True)

        def loop_body(s, _):
            body(s, True, True, True)
            return None
        with sc('s6_loop'):
            jax.lax.fori_loop(1 if nopeel else 2, NL * NC, loop_body, None)
        with sc('s7_epi'):
            body(NL * NC, False, True, False)
        with sc('s8_fin'):
            for c in range(NC):
                out_copy(c).wait()

    return kernel


def build(**cfg):
    cfg = dict(cfg)
    flags = cfg.pop("flags", None)
    wdpad = cfg.pop("wdpad", 16)
    xbpad = cfg.pop("xbpad", 0)
    useC = cfg.pop("useC", 1)
    qpad = cfg.pop("qpad", 16)
    pads = cfg.pop("pads", {})
    T = cfg.get("T", 256)
    shapes = dict(
        xin=pltpu.VMEM((D, S), BF16), xa=pltpu.VMEM((D, S), F32), xb=pltpu.VMEM((D, S), F32),
        outs=pltpu.VMEM((D, S), BF16), wqkv_raw=pltpu.VMEM((D, 3 * D), BF16), wo_raw=pltpu.VMEM((D, D), BF16),
        w32=pltpu.VMEM((5, 1792, 128), F32), wqkvP=pltpu.VMEM((3 * D, DP), BF16), woTP=pltpu.VMEM((D, DP), BF16),
        wg=pltpu.VMEM((D, DF), BF16), wu=pltpu.VMEM((D, DF), BF16), wdT=pltpu.VMEM((D + wdpad, DF), BF16),
        q=pltpu.VMEM((5, T + qpad, 128), F32), k=pltpu.VMEM((5, T + PAD, 128), F32), v=pltpu.VMEM((5, T + PAD, 128), F32),
        xnA=pltpu.VMEM((T, D), BF16), xnB=pltpu.VMEM((T + xbpad, D), BF16), xnC=pltpu.VMEM((T if useC else 16, D), BF16),
        o=pltpu.VMEM((T, DP), BF16), zs=pltpu.SMEM((1,), jnp.int32),
        sems=pltpu.SemaphoreType.DMA((16,)), osem=pltpu.SemaphoreType.DMA(()))
    names, scratch = [], []
    for n in ORDER + ["end"]:
        if pads.get(n):
            names.append("pad_" + n)
            scratch.append(pltpu.VMEM((8 * pads[n], 128), F32))
        if n != "end" and not (n == "xnC" and useC < 0):
            names.append(n)
            scratch.append(shapes[n])
    kern = make_kernel(names, **cfg)

    @jax.jit
    def fn(A_x, A_wqkv, A_wo, B_x, B_w_gate, B_w_up, B_w_down):
        xT = A_x.reshape(S, D).T
        wdT = B_w_down.T
        hbm = pl.BlockSpec(memory_space=pltpu.HBM)
        outT = pl.pallas_call(
            kern,
            out_shape=jax.ShapeDtypeStruct((D, S), BF16),
            in_specs=[hbm] * 6,
            out_specs=hbm,
            scratch_shapes=scratch,
            compiler_params=pltpu.CompilerParams(vmem_limit_bytes=110 * 1024 * 1024, flags=flags),
        )(xT, A_wqkv, A_wo, B_w_gate, B_w_up, wdT)
        return outT.T.reshape(1, S, D)
    return fn


_kernel_fn = build()


@jax.jit
def pallas_interleave_layers__sliding_local_dilated__glu_gated_geglu__prompt_kernel(
    A_x: jax.Array,
    A_wqkv: jax.Array,
    A_wo: jax.Array,
    B_x: jax.Array,
    B_w_gate: jax.Array,
    B_w_up: jax.Array,
    B_w_down: jax.Array,
):
    return _kernel_fn(A_x, A_wqkv, A_wo, B_x, B_w_gate, B_w_up, B_w_down)
```

```python
import jax
import jax.numpy as jnp
import jax.experimental.pallas as pl
import jax.experimental.pallas.tpu as pltpu

S, D, DP = 2048, 576, 640
H, DH, W, DIL = 32, 18, 8, 2
DF, NL = 4608, 2
T, FB, RS = 256, 1536, 16
NC, NF, NSB = S // T, DF // FB, T // RS
PAD = 16
ATT_SPAN = 0.66
NEG = -1e30
LOG2E = 1.4426950408889634
F32, BF16 = jnp.float32, jnp.bfloat16
NT = (((1,), (1,)), ((), ()))


def _ln_rows(x):
    m = jnp.mean(x, axis=0, keepdims=True)
    xc = x - m
    v = jnp.mean(xc * xc, axis=0, keepdims=True)
    return (xc * jax.lax.rsqrt(v + 1e-5)).T.astype(BF16)


def _gelu(x):
    c = 0.7978845608028654
    return 0.5 * x * (1.0 + jnp.tanh(c * (x + 0.044715 * (x * x * x))))


def _kernel(xT_hbm, wqkv_hbm, wo_hbm, wg_hbm, wu_hbm, wdT_hbm, outT_hbm,
            xin, xa, xb, outs, wqkv_raw, wo_raw, w32, wqkvP, woTP, wg, wu, wdT,
            q_s, k_s, v_s, xnA, xnB, o_s, zs, sems, osem):
    def cp_cols(src, dst, c0, n, sem):
        return pltpu.make_async_copy(src.at[:, pl.ds(c0, n)], dst.at[pl.ds(0, D), pl.ds(c0, n)], sem)

    cp_x0 = cp_cols(xT_hbm, xin, 0, T, sems.at[0])
    cp_x1 = cp_cols(xT_hbm, xin, T, T, sems.at[1])
    cp_x2 = cp_cols(xT_hbm, xin, 2 * T, S - 2 * T, sems.at[2])
    cp_q = [cp_cols(wqkv_hbm, wqkv_raw, c0, n, sems.at[3 + i])
            for i, (c0, n) in enumerate([(0, 640), (640, 512), (1152, 576)])]
    cp_wo = pltpu.make_async_copy(wo_hbm, wo_raw, sems.at[6])
    cp_g = [cp_cols(wg_hbm, wg, f * FB, FB, sems.at[7 + 3 * f]) for f in range(NF)]
    cp_u = [cp_cols(wu_hbm, wu, f * FB, FB, sems.at[8 + 3 * f]) for f in range(NF)]
    cp_d = [cp_cols(wdT_hbm, wdT, f * FB, FB, sems.at[9 + 3 * f]) for f in range(NF)]
    for c in [cp_x0, cp_q[0], cp_q[1], cp_q[2], cp_wo, cp_x1, cp_x2, cp_g[0], cp_u[0],
              cp_g[1], cp_u[1], cp_d[0], cp_g[2], cp_u[2], cp_d[1], cp_d[2]]:
        c.start()

    def out_copy(c):
        c0 = pl.multiple_of(c * T, T)
        return pltpu.make_async_copy(outs.at[:, pl.ds(c0, T)], outT_hbm.at[:, pl.ds(c0, T)], osem)

    def cvt(c):
        xb[:, c * T:(c + 1) * T] = xin[:, c * T:(c + 1) * T].astype(F32)

    zs[0] = 0
    for j in range(5):
        for r in (0, T):
            k_s[j, pl.ds(r, PAD), :] = jnp.zeros((PAD, 128), F32)
            v_s[j, pl.ds(r, PAD), :] = jnp.zeros((PAD, 128), F32)

    def transpose_blocks(j0, j1):
        for j in range(j0, j1):
            ncol = min(128, 3 * D - j * 128)
            blk = wqkv_raw[:, j * 128:j * 128 + ncol].astype(F32)
            if ncol < 128:
                blk = jnp.concatenate([blk, jnp.zeros((D, 128 - ncol), F32)], axis=1)
            blk = jnp.concatenate([blk, jnp.zeros((DP - D, 128), F32)], axis=0)
            for t in range(5):
                w32[t, pl.ds(j * 128, 128), :] = blk[t * 128:(t + 1) * 128, :].T

    def permute_part(p):
        for d in range(DH):
            dst = (p * 16 + d) if d < 16 else (48 + p * 2 + d - 16)
            for t in range(5):
                rows = w32[t, pl.ds(p * D + d, H, stride=DH), :]
                wqkvP[pl.ds(dst * H, H), t * 128:(t + 1) * 128] = rows.astype(BF16)

    def prep_wo():
        for t in range(5):
            ncol = min(128, D - t * 128)
            blk = wo_raw[:, t * 128:t * 128 + ncol].astype(F32)
            if ncol < 128:
                blk = jnp.concatenate([blk, jnp.zeros((D, 128 - ncol), F32)], axis=1)
            w32[t, pl.ds(0, D), :] = blk
            for d in range(DH):
                w32[t, pl.ds(D + d * H, H), :] = w32[t, pl.ds(d, H, stride=DH), :]
            w32[t, pl.ds(2 * D, 64), :] = jnp.zeros((64, 128), F32)
            for j in range(5):
                pb = w32[t, pl.ds(D + j * 128, 128), :]
                woTP[pl.ds(t * 128, ncol), j * 128:(j + 1) * 128] = pb.T[0:ncol, :].astype(BF16)

    lo_mask = jax.lax.broadcasted_iota(jnp.int32, (T, 128), 1) < 64
    cs = LOG2E * DH ** -0.5

    def proj(r0, n):
        return jax.lax.dot_general(xnA[...], wqkvP[pl.ds(r0, n), 0:D], NT, preferred_element_type=F32)

    def store_main(ref, r, c0, val, scale=None):
        for j in range(4):
            v = val[:, c0 + j * 128:c0 + (j + 1) * 128]
            ref[j, pl.ds(r, T), :] = v if scale is None else v * scale

    def store_qk_tail(t):
        q_s[4, pl.ds(0, T), :] = jnp.where(lo_mask, t * cs, 0.0)
        k_s[4, pl.ds(PAD, T), :] = pltpu.roll(t, 64, axis=1)

    def store_v_tail(t):
        v_s[4, pl.ds(PAD, T), :] = jnp.concatenate([t, jnp.zeros((T, 64), F32)], axis=1)

    def qkv_part(c0):
        keep = c0 > 0
        for j in range(5):
            k_s[j, pl.ds(0, PAD), :] = jnp.where(keep, k_s[j, pl.ds(T, PAD), :], 0.0)
            v_s[j, pl.ds(0, PAD), :] = jnp.where(keep, v_s[j, pl.ds(T, PAD), :], 0.0)
        qkv = proj(0, 3 * D)
        store_main(q_s, 0, 0, qkv, cs)
        store_main(k_s, PAD, 512, qkv)
        store_main(v_s, PAD, 1024, qkv)
        store_qk_tail(qkv[:, 1536:1664])
        store_v_tail(qkv[:, 1664:1728])

    def att_block(c0, sb):
        base = sb * RS
        q = [q_s[j, pl.ds(base, RS), :] for j in range(5)]
        logits = []
        for w in range(W):
            o0 = base + PAD - DIL * w
            s = q[0] * k_s[0, pl.ds(o0, RS), :]
            for j in range(1, 5):
                s = s + q[j] * k_s[j, pl.ds(o0, RS), :]
            s = s + pltpu.roll(s, 64, axis=1)
            s = s + pltpu.roll(s, 32, axis=1)
            if base < DIL * w:
                row = jax.lax.broadcasted_iota(jnp.int32, (RS, 128), 0) + (base + c0)
                s = jnp.where(row >= DIL * w, s, NEG)
            logits.append(s)
        m = logits[0]
        for w in range(1, W):
            m = jnp.maximum(m, logits[w])
        es = [jnp.exp2(l - m) for l in logits]
        den = es[0]
        for w in range(1, W):
            den = den + es[w]
        inv = 1.0 / den
        for j in range(5):
            o = es[0] * v_s[j, pl.ds(base + PAD, RS), :]
            for w in range(1, W):
                o = o + es[w] * v_s[j, pl.ds(base + PAD - DIL * w, RS), :]
            o_s[pl.ds(base, RS), j * 128:(j + 1) * 128] = (o * inv).astype(BF16)

    def att_tail(a0):
        yT = jax.lax.dot_general(woTP[:, 0:D], o_s[:, 0:D], NT, preferred_element_type=F32)
        xa[:, pl.ds(a0, T)] = xb[:, pl.ds(a0, T)] + yT

    def pin_q(val):
        q_s[0, pl.ds(pl.multiple_of(T + zs[0], 8), 8), :] = val

    def pin_d(val):
        wdT[pl.ds(pl.multiple_of(D + zs[0], 16), 16), 0:128] = val

    def fence(ref):
        return ref[pl.ds(pl.multiple_of(zs[0], 16), 16), 0:128]

    def step(s, do_att, first=False):
        if do_att:
            a0 = pl.multiple_of((s % NC) * T, T)
            n0 = pl.multiple_of(((s + 1) % NC) * T, T)
            qkv_part(a0)
        b0 = pl.multiple_of(((s - 1) % NC) * T, T)
        acc = xa[:, pl.ds(b0, T)]
        xnB[...] = _ln_rows(acc)
        hs = {}

        def gate_up(f):
            if first:
                cp_g[f].wait()
                cp_u[f].wait()
            x = xnB[...]
            g = jnp.dot(x, wg[:, f * FB:(f + 1) * FB], preferred_element_type=F32)
            u = jnp.dot(x, wu[:, f * FB:(f + 1) * FB], preferred_element_type=F32)
            hs[f] = (_gelu(g) * u).astype(BF16)
            if do_att:
                for sb in range(NSB):
                    pos = ATT_SPAN * NF * sb / NSB
                    if int(pos) == f:
                        col = int((pos - f) * FB) // 128 * 128
                        pin_q(g[0:8, col:col + 128])
                        att_block(a0, sb)
                        if sb == NSB - 1:
                            att_tail(a0)

        def down(f, acc):
            if do_att and f == 0:
                xnA[...] = _ln_rows(xb[:, pl.ds(n0, T)])
                pin_d(fence(xnA))
            if first and f < 2:
                for c in ([cp_d[0]], [cp_d[1], cp_d[2]])[f]:
                    c.wait()
            return acc + jax.lax.dot_general(wdT[pl.ds(0, D), f * FB:(f + 1) * FB], hs[f], NT,
                                             preferred_element_type=F32)

        if first:
            gate_up(0)
            gate_up(1)
            for c in range(4, NC):
                cvt(c)
            acc = down(0, acc)
            gate_up(2)
            acc = down(2, down(1, acc))
        else:
            for f in range(NF):
                gate_up(f)
                acc = down(f, acc)
        xb[:, pl.ds(b0, T)] = acc
        outs[:, pl.ds(b0, T)] = acc.astype(BF16)

        @pl.when(s - 1 >= (NL - 1) * NC)
        def _():
            out_copy(s - 1 - (NL - 1) * NC).start()

    cp_x0.wait()
    cvt(0)
    xnA[...] = _ln_rows(xb[:, 0:T])
    cp_q[0].wait()
    transpose_blocks(0, 5)
    permute_part(0)
    cp_q[1].wait()
    store_main(q_s, 0, 0, proj(0, 512), cs)
    transpose_blocks(5, 9)
    permute_part(1)
    cp_q[2].wait()
    store_main(k_s, PAD, 0, proj(512, 512))
    store_qk_tail(proj(1536, 128))
    transpose_blocks(9, 14)
    permute_part(2)
    cp_wo.wait()
    cp_x1.wait()
    store_main(v_s, PAD, 0, proj(1024, 512))
    store_v_tail(proj(1664, 64))
    prep_wo()
    cvt(1)
    xnA[...] = _ln_rows(xb[:, T:2 * T])
    pin_q(fence(xnA).astype(F32)[0:8, :])
    for sb in range(NSB):
        att_block(0, sb)
    att_tail(0)

    cp_x2.wait()

    def cvt_dyn(i, _):
        c0 = pl.multiple_of(i * T, T)
        xb[:, pl.ds(c0, T)] = xin[:, pl.ds(c0, T)].astype(F32)
    jax.lax.fori_loop(2, 4, cvt_dyn, None)

    step(1, True, first=True)
    jax.lax.fori_loop(2, NL * NC, lambda s, _: step(s, True), None)
    step(NL * NC, False)
    for c in range(NC):
        out_copy(c).wait()


def build(**cfg):
    @jax.jit
    def fn(A_x, A_wqkv, A_wo, B_x, B_w_gate, B_w_up, B_w_down):
        hbm = pl.BlockSpec(memory_space=pltpu.HBM)
        outT = pl.pallas_call(
            _kernel,
            out_shape=jax.ShapeDtypeStruct((D, S), BF16),
            in_specs=[hbm] * 6,
            out_specs=hbm,
            scratch_shapes=[
                pltpu.VMEM((D, S), BF16),
                pltpu.VMEM((D, S), F32),
                pltpu.VMEM((D, S), F32),
                pltpu.VMEM((D, S), BF16),
                pltpu.VMEM((D, 3 * D), BF16),
                pltpu.VMEM((D, D), BF16),
                pltpu.VMEM((5, 1792, 128), F32),
                pltpu.VMEM((3 * D, DP), BF16),
                pltpu.VMEM((D, DP), BF16),
                pltpu.VMEM((D, DF), BF16),
                pltpu.VMEM((D, DF), BF16),
                pltpu.VMEM((D + 16, DF), BF16),
                pltpu.VMEM((5, T + 16, 128), F32),
                pltpu.VMEM((5, T + PAD, 128), F32),
                pltpu.VMEM((5, T + PAD, 128), F32),
                pltpu.VMEM((T, D), BF16),
                pltpu.VMEM((T, D), BF16),
                pltpu.VMEM((T, DP), BF16),
                pltpu.SMEM((1,), jnp.int32),
                pltpu.SemaphoreType.DMA((16,)),
                pltpu.SemaphoreType.DMA(()),
            ],
            compiler_params=pltpu.CompilerParams(vmem_limit_bytes=110 * 1024 * 1024),
        )(A_x.reshape(S, D).T, A_wqkv, A_wo, B_w_gate, B_w_up, B_w_down.T)
        return outT.T.reshape(1, S, D)
    return fn


_kernel_fn = build()


@jax.jit
def pallas_interleave_layers__sliding_local_dilated__glu_gated_geglu__prompt_kernel(
    A_x: jax.Array,
    A_wqkv: jax.Array,
    A_wo: jax.Array,
    B_x: jax.Array,
    B_w_gate: jax.Array,
    B_w_up: jax.Array,
    B_w_down: jax.Array,
):
    return _kernel_fn(A_x, A_wqkv, A_wo, B_x, B_w_gate, B_w_up, B_w_down)
```
